```python
import os as _os
_os.environ.setdefault("JAX_PLATFORMS", "cpu")
import jax
import jax.numpy as jnp

def _softmax(x, axis=-1):
    return jax.nn.softmax(x, axis=axis)
def _gelu(x):
    return jax.nn.gelu(x, approximate=True)
def _silu(x):
    return jax.nn.silu(x)
def _sigmoid(x):
    return jax.nn.sigmoid(x)
def _layernorm(x, axis=-1, eps=1e-5):
    m = jnp.mean(x, axis=axis, keepdims=True)
    v = jnp.var(x, axis=axis, keepdims=True)
    return (x - m) / jnp.sqrt(v + eps)
def _scatter_add(tgt, idx, src, axis=0):
    return tgt.at[idx].add(src)
def _segment_sum(src, seg, n):
    return jax.ops.segment_sum(src, seg, n)
class _Rng:
    def __init__(self, key):
        self._k = key
    def _next(self):
        self._k, sub = jax.random.split(self._k)
        return sub
    def normal(self, shape):
        return jax.random.normal(self._next(), shape, dtype=jnp.bfloat16)
    def randint(self, lo, hi, shape):
        return jax.random.randint(self._next(), shape, lo, hi, dtype=jnp.int32)
    def uniform(self, shape, lo=0.0, hi=1.0):
        return jax.random.uniform(self._next(), shape, jnp.bfloat16, lo, hi)
    def permutation(self, n):
        return jax.random.permutation(self._next(), n)


kernel_name = 'standalone__sliding_local_fixed_window__prompt'

def setup_inputs():
    _rng = _Rng(jax.random.key(int.from_bytes(__import__("os").urandom(4), "little")))
    _w = (lambda a: (lambda t: t.astype(jnp.bfloat16) if jnp.issubdtype(t.dtype, jnp.floating) else t)(jnp.asarray(a)))
    B, H, S, D = 1, 32, 2048, 128
    return {
        "q": _w((lambda *s: _rng.normal(s) * 0.4)(B, H, S, D)),
        "k": _w((lambda *s: _rng.normal(s) * 0.4)(B, H, S, D)),
        "v": _w((lambda *s: _rng.normal(s) * 0.05)(B, H, S, D)),
    }

def reference(q, k, v):
    B, H, S, D = q.shape
    w = 32
    pos = jnp.arange(S)
    rel = pos[:, None] - pos[None, :]
    mask = (rel >= 0) & (rel < w)
    scores = jnp.einsum("bhqd,bhkd->bhqk", q, k) * (D ** -0.5)
    scores = jnp.where(mask[None, None], scores, (lambda x, dt: x.astype(dt))(jnp.array(-1e9), q.dtype))
    p = _softmax(scores, axis=-1)
    return jnp.einsum("bhqk,bhkd->bhqd", p, v)
```

```python
import math

import jax
import jax.numpy as jnp
import jax.experimental.pallas as pl
import jax.experimental.pallas.tpu as pltpu

_W = 32
_T = 128
_NEG = -1e30
_BIG = 3.0e38


def _head(q_ref, k_ref, v_ref, o_ref, cap_ref, base, seq, c):
    nt = seq // _T
    row = jax.lax.broadcasted_iota(jnp.int32, (_W, _T), 0)
    col = jax.lax.broadcasted_iota(jnp.int32, (_W, _T), 1)
    lower = col <= row

    def rows(j, n):
        return pl.ds(pl.multiple_of(base + j * _T, _T), n)

    def qk(j):
        m = _T + _W if j < nt - 1 else _T
        return jax.lax.dot_general(
            q_ref[rows(j, m), :], k_ref[rows(j, _T), :],
            (((1,), (1,)), ((), ())), preferred_element_type=jnp.float32)

    def softmax(a, aprev):
        top = jnp.where(lower, a[:_W], _NEG if aprev is None else aprev[_T:])
        s = jnp.concatenate([top, a[_W:_T]], 0) * c
        s = jnp.minimum(s, cap_ref[...])
        p = jnp.exp2(s - jnp.max(s, axis=-1, keepdims=True))
        r = 1.0 / jnp.sum(p, axis=-1, keepdims=True)
        pcur = jnp.concatenate([jnp.where(lower, p[:_W], 0.0), p[_W:]], 0)
        pprev = jnp.where(lower, 0.0, p[:_W])
        return pcur.astype(v_ref.dtype), pprev.astype(v_ref.dtype), r

    a = qk(0)
    pcur, _, r = softmax(a, None)
    carry = None
    for j in range(nt):
        lhs = pcur
        if j < nt - 1:
            an = qk(j + 1)
            pcur_n, pprev_n, r_n = softmax(an, a)
            lhs = jnp.concatenate([pcur, pprev_n], 0)
        b = jnp.dot(lhs, v_ref[rows(j, _T), :], preferred_element_type=jnp.float32)
        o = b[:_T]
        if carry is not None:
            o = jnp.concatenate([o[:_W] + carry, o[_W:]], 0)
        o_ref[rows(j, _T), :] = (o * r).astype(o_ref.dtype)
        if j < nt - 1:
            carry = b[_T:]
            a, pcur, r = an, pcur_n, r_n


@jax.jit
def pallas_standalone__sliding_local_fixed_window__prompt_kernel(
    q: jax.Array,
    k: jax.Array,
    v: jax.Array,
):
    B, H, S, D = q.shape
    NH = B * H
    c = float(D ** -0.5 * math.log2(math.e))
    AH = 2

    def kern(q_hbm, k_hbm, v_hbm, o_hbm, qb, kb, vb, ob, cap_ref, isem, osem):
        def cin(h):
            sl = pl.ds(pl.multiple_of(h * S, S), S)
            s = h % AH
            return [pltpu.make_async_copy(q_hbm.at[sl], qb.at[sl], isem.at[0, s]),
                    pltpu.make_async_copy(k_hbm.at[sl], kb.at[sl], isem.at[1, s]),
                    pltpu.make_async_copy(v_hbm.at[sl], vb.at[sl], isem.at[2, s])]

        for h in range(AH):
            for cp in cin(h):
                cp.start()
        row = jax.lax.broadcasted_iota(jnp.int32, (_T, _T), 0)
        col = jax.lax.broadcasted_iota(jnp.int32, (_T, _T), 1)
        cap_ref[...] = jnp.where(((row - col) & (_T - 1)) < _W, _BIG, _NEG).astype(jnp.float32)
        n = (NH - 1) * S
        bulk = pltpu.make_async_copy(ob.at[pl.ds(0, n)], o_hbm.at[pl.ds(0, n)], osem.at[0])
        last = pltpu.make_async_copy(ob.at[pl.ds(n, S)], o_hbm.at[pl.ds(n, S)], osem.at[1])

        def body(h, _):
            for cp in cin(h):
                cp.wait()

            @pl.when(h + AH < NH)
            def _():
                for cp in cin(h + AH):
                    cp.start()

            @pl.when(h == NH - 1)
            def _():
                bulk.start()

            _head(qb, kb, vb, ob, cap_ref, h * S, S, c)

        jax.lax.fori_loop(0, NH, body, None)
        last.start()
        bulk.wait()
        last.wait()

    q2, k2, v2 = (x.reshape(NH * S, D) for x in (q, k, v))
    buf = pltpu.VMEM((NH * S, D), q.dtype)
    hbm = pl.BlockSpec(memory_space=pl.ANY)
    o = pl.pallas_call(
        kern,
        in_specs=[hbm] * 3,
        out_specs=hbm,
        out_shape=jax.ShapeDtypeStruct(q2.shape, q.dtype),
        scratch_shapes=[buf, buf, buf, buf, pltpu.VMEM((_T, _T), jnp.float32),
                        pltpu.SemaphoreType.DMA((3, AH)), pltpu.SemaphoreType.DMA((2,))],
        compiler_params=pltpu.CompilerParams(vmem_limit_bytes=100 << 20),
    )(q2, k2, v2)
    return o.reshape(q.shape)
```

```python
import math

import jax
import jax.numpy as jnp
import jax.experimental.pallas as pl
import jax.experimental.pallas.tpu as pltpu

_W = 32
_T = 128
_READ_ROWS = 1024
_AHEAD = 2
_WRITE_ROWS = 32
_WRITES_PER_HEAD = 14
_WRITES_IN_FLIGHT = 6


def _attend_head(q_ref, k_ref, v_ref, o_ref, cap_ref, h, scale_log2e):
    n_tiles = q_ref.shape[1] // _T
    row = jax.lax.broadcasted_iota(jnp.int32, (_W, _T), 0)
    col = jax.lax.broadcasted_iota(jnp.int32, (_W, _T), 1)
    own_tile = col <= row

    def scores(j):
        n = _T + _W if j < n_tiles - 1 else _T
        return jax.lax.dot_general(
            q_ref[h, pl.ds(j * _T, n), :], k_ref[h, pl.ds(j * _T, _T), :],
            (((1,), (1,)), ((), ())), preferred_element_type=jnp.float32)

    def softmax(cur, prev):
        top = jnp.where(own_tile, cur[:_W], -jnp.inf if prev is None else prev[_T:])
        s = jnp.concatenate([top, cur[_W:_T]], 0) * scale_log2e
        s = jnp.minimum(s, cap_ref[...])
        p = jnp.exp2(s - jnp.max(s, axis=-1, keepdims=True))
        inv = 1.0 / jnp.sum(p, axis=-1, keepdims=True)
        p_own = jnp.concatenate([jnp.where(own_tile, p[:_W], 0.0), p[_W:]], 0)
        p_prev = jnp.where(own_tile, 0.0, p[:_W])
        return p_own.astype(v_ref.dtype), p_prev.astype(v_ref.dtype), inv

    s_cur = scores(0)
    p_own, _, inv = softmax(s_cur, None)
    carry = None
    for j in range(n_tiles):
        last = j == n_tiles - 1
        lhs = p_own
        if not last:
            s_next = scores(j + 1)
            p_own_next, p_prev_next, inv_next = softmax(s_next, s_cur)
            lhs = jnp.concatenate([p_own, p_prev_next], 0)
        pv = jnp.dot(lhs, v_ref[h, pl.ds(j * _T, _T), :],
                     preferred_element_type=jnp.float32)
        acc = pv[:_T]
        if carry is not None:
            acc = jnp.concatenate([acc[:_W] + carry, acc[_W:]], 0)
        o_ref[h, pl.ds(j * _T, _T), :] = (acc * inv).astype(o_ref.dtype)
        if not last:
            carry = pv[_T:]
            s_cur, p_own, inv = s_next, p_own_next, inv_next


def _kernel(q_hbm, k_hbm, v_hbm, o_hbm, q_vm, k_vm, v_vm, o_vm, cap_ref,
            in_sems, out_sem):
    n_heads, seq, dim = q_hbm.shape
    scale_log2e = float(dim ** -0.5 * math.log2(math.e))
    reads_per_head = 3 * (seq // _READ_ROWS)
    group = n_heads // 2
    writes_per_group = seq // _WRITE_ROWS
    n_writes = 2 * writes_per_group
    n_early = _AHEAD * _WRITES_PER_HEAD
    tail = n_heads - _AHEAD
    assert seq % _READ_ROWS == 0 and n_heads % 2 == 0
    assert group <= tail and _WRITES_IN_FLIGHT <= n_early <= writes_per_group

    def read(h, i):
        src, dst = ((q_hbm, q_vm), (k_hbm, k_vm), (v_hbm, v_vm))[i % 3]
        idx = (h, pl.ds((i // 3) * _READ_ROWS, _READ_ROWS))
        return pltpu.make_async_copy(src.at[idx], dst.at[idx], in_sems.at[h % _AHEAD])

    def start_reads(h):
        for i in range(reads_per_head):
            read(h, i).start(priority=i % 2)

    def write(g, r):
        idx = (pl.ds(g * group, group), pl.ds(r, _WRITE_ROWS))
        return pltpu.make_async_copy(o_vm.at[idx], o_hbm.at[idx], out_sem)

    for h in range(_AHEAD):
        start_reads(h)

    row = jax.lax.broadcasted_iota(jnp.int32, (_T, _T), 0)
    col = jax.lax.broadcasted_iota(jnp.int32, (_T, _T), 1)
    cap_ref[...] = jnp.where(((row - col) & (_T - 1)) < _W, jnp.inf, -jnp.inf)

    def head_step(h, _):
        @pl.when(h < tail)
        def _():
            for i in range(reads_per_head):
                read(h, i).wait()
            start_reads(h + _AHEAD)

        @pl.when(h == tail)
        def _():
            pending = [(t, i) for t in range(tail, n_heads)
                       for i in range(reads_per_head)]
            for t, i in pending[:-1]:
                read(t, i).wait()
            for i in range(_WRITES_PER_HEAD):
                write(0, i * _WRITE_ROWS).start()
            read(*pending[-1]).wait()

        for n in range(1, _AHEAD):
            @pl.when(h == tail + n)
            def _():
                for i in range(n * _WRITES_PER_HEAD, (n + 1) * _WRITES_PER_HEAD):
                    write(0, i * _WRITE_ROWS).start()

        _attend_head(q_vm, k_vm, v_vm, o_vm, cap_ref, h, scale_log2e)

    jax.lax.fori_loop(0, n_heads, head_step, None)

    def wait_write(i, _):
        write(0, 0).wait()

    def next_write(i, _):
        r = pl.multiple_of(jax.lax.rem(i, writes_per_group) * _WRITE_ROWS, _WRITE_ROWS)
        write(jax.lax.div(i, writes_per_group), r).start()
        write(0, 0).wait()

    jax.lax.fori_loop(0, n_early - _WRITES_IN_FLIGHT + 1, wait_write, None)
    jax.lax.fori_loop(n_early, n_writes, next_write, None)
    jax.lax.fori_loop(0, _WRITES_IN_FLIGHT - 1, wait_write, None)


@jax.jit
def pallas_standalone__sliding_local_fixed_window__prompt_kernel(
    q: jax.Array,
    k: jax.Array,
    v: jax.Array,
):
    B, H, S, D = q.shape
    shape = (B * H, S, D)
    hbm = pl.BlockSpec(memory_space=pl.ANY)
    out = pl.pallas_call(
        _kernel,
        in_specs=[hbm, hbm, hbm],
        out_specs=hbm,
        out_shape=jax.ShapeDtypeStruct(shape, v.dtype),
        scratch_shapes=[
            pltpu.VMEM(shape, q.dtype),
            pltpu.VMEM(shape, k.dtype),
            pltpu.VMEM(shape, v.dtype),
            pltpu.VMEM(shape, v.dtype),
            pltpu.VMEM((_T, _T), jnp.float32),
            pltpu.SemaphoreType.DMA((_AHEAD,)),
            pltpu.SemaphoreType.DMA(()),
        ],
        compiler_params=pltpu.CompilerParams(vmem_limit_bytes=100 << 20),
    )(q.reshape(shape), k.reshape(shape), v.reshape(shape))
    return out.reshape(B, H, S, D)
```
